```python
import os as _os
_os.environ.setdefault("JAX_PLATFORMS", "cpu")
import jax
import jax.numpy as jnp

def _softmax(x, axis=-1):
    return jax.nn.softmax(x, axis=axis)
def _gelu(x):
    return jax.nn.gelu(x, approximate=True)
def _silu(x):
    return jax.nn.silu(x)
def _sigmoid(x):
    return jax.nn.sigmoid(x)
def _layernorm(x, axis=-1, eps=1e-5):
    m = jnp.mean(x, axis=axis, keepdims=True)
    v = jnp.var(x, axis=axis, keepdims=True)
    return (x - m) / jnp.sqrt(v + eps)
def _scatter_add(tgt, idx, src, axis=0):
    return tgt.at[idx].add(src)
def _segment_sum(src, seg, n):
    return jax.ops.segment_sum(src, seg, n)
class _Rng:
    def __init__(self, key):
        self._k = key
    def _next(self):
        self._k, sub = jax.random.split(self._k)
        return sub
    def normal(self, shape):
        return jax.random.normal(self._next(), shape, dtype=jnp.bfloat16)
    def randint(self, lo, hi, shape):
        return jax.random.randint(self._next(), shape, lo, hi, dtype=jnp.int32)
    def uniform(self, shape, lo=0.0, hi=1.0):
        return jax.random.uniform(self._next(), shape, jnp.bfloat16, lo, hi)
    def permutation(self, n):
        return jax.random.permutation(self._next(), n)


kernel_name = 'parallel_sum__ssm_conv_s5__geglu_ffn__prompt'

def setup_inputs():
    _rng = _Rng(jax.random.key(int.from_bytes(__import__("os").urandom(4), "little")))
    _w = (lambda a: (lambda t: t.astype(jnp.bfloat16) if jnp.issubdtype(t.dtype, jnp.floating) else t)(jnp.asarray(a)))
    def _A_setup():
        B, S, D = 1, 2048, 512
        P = D
        Lambda_re = -0.5 * jnp.exp((lambda *s: _rng.normal(s) * 0.8)(P))
        Lambda_im = (lambda *s: _rng.normal(s) * 0.8)(P) * 1.0
        B_re = (lambda *s: _rng.normal(s) * 0.8)(P, D) * (D ** -0.5)
        B_im = (lambda *s: _rng.normal(s) * 0.8)(P, D) * (D ** -0.5)
        C_re = (lambda *s: _rng.normal(s) * 0.8)(D, P) * (P ** -0.5)
        C_im = (lambda *s: _rng.normal(s) * 0.8)(D, P) * (P ** -0.5)
        log_dt = (lambda *s: _rng.normal(s) * 0.8)(P) * 0.3 - 2.0
        Dskip = (lambda *s: _rng.normal(s) * 0.8)(D)
        return {
            "x": _w((lambda *s: _rng.normal(s) * 0.05)(B, S, D)),
            "Lambda_re": _w(Lambda_re),
            "Lambda_im": _w(Lambda_im),
            "B_re": _w(B_re),
            "B_im": _w(B_im),
            "C_re": _w(C_re),
            "C_im": _w(C_im),
            "log_dt": _w(log_dt),
            "Dskip": _w(Dskip),
        }
    _A_in = _A_setup()

    def _B_setup():
        B, S, D, F = 1, 2048, 512, 1376
        return {
            "x": _w((lambda *s: _rng.normal(s) * 0.05)(B, S, D)),
            "w_gate": _w((lambda *s: _rng.normal(s) * 0.05)(D, F)),
            "w_up": _w((lambda *s: _rng.normal(s) * 0.05)(D, F)),
            "w_down": _w((lambda *s: _rng.normal(s) * 0.05)(F, D)),
        }
    _B_in = _B_setup()

    return {
        "A_x": _A_in["x"],
        "A_Lambda_re": _A_in["Lambda_re"],
        "A_Lambda_im": _A_in["Lambda_im"],
        "A_B_re": _A_in["B_re"],
        "A_B_im": _A_in["B_im"],
        "A_C_re": _A_in["C_re"],
        "A_C_im": _A_in["C_im"],
        "A_log_dt": _A_in["log_dt"],
        "A_Dskip": _A_in["Dskip"],
        "B_x": _B_in["x"],
        "B_w_gate": _B_in["w_gate"],
        "B_w_up": _B_in["w_up"],
        "B_w_down": _B_in["w_down"],
    }

def reference(A_x, A_Lambda_re, A_Lambda_im, A_B_re, A_B_im, A_C_re, A_C_im, A_log_dt, A_Dskip, B_x, B_w_gate, B_w_up, B_w_down):
    def _A_ref(x, Lambda_re, Lambda_im, B_re, B_im, C_re, C_im, log_dt, Dskip):
        Bsz, L, H = x.shape
        Lam = Lambda_re + 1j * Lambda_im
        Bmat = B_re + 1j * B_im
        Cmat = C_re + 1j * C_im
        dt = jnp.exp(log_dt)
        Lam_bar = jnp.exp(dt * Lam)
        B_bar = ((Lam_bar - 1.0) / Lam)[:, None] * Bmat
        Bu = jnp.einsum("bld,pd->blp", x + 0j, B_bar)
        h = jnp.zeros_like(Bu[:, 0, :])
        hs = []
        for t in range(L):
            h = Lam_bar[None, :] * h + Bu[:, t, :]
            hs.append(h)
        hseq = jnp.stack(hs, 1)
        y = 2.0 * jnp.einsum("blp,dp->bld", hseq, Cmat).real + x * Dskip[None, None, :]
        return y

    def _B_ref(x, w_gate, w_up, w_down):
        return (_gelu(x @ w_gate) * (x @ w_up)) @ w_down

    x = A_x
    xn = _layernorm(x, axis=-1)
    return x + _A_ref(xn, A_Lambda_re, A_Lambda_im, A_B_re, A_B_im, A_C_re, A_C_im, A_log_dt, A_Dskip) + _B_ref(xn, B_w_gate, B_w_up, B_w_down)
```

```python
import functools
import jax
import jax.numpy as jnp
import numpy as np
from jax.experimental import pallas as pl
from jax.experimental.pallas import tpu as pltpu

L, D, P, F = 2048, 512, 512, 1376
f32, bf16 = jnp.float32, jnp.bfloat16
NT = (((1,), (1,)), ((), ()))

def _rb(v):
    return v.astype(bf16).astype(f32)

def _cmul(ar, ai, br, bi):
    return ar * br - ai * bi, ar * bi + ai * br

def make(Tb=512, interpret=False):
    NB = L // Tb
    Tc = Tb // 8
    SY = Tc + 1

    def kernel(x_ref, lre_ref, lim_ref, ldt_ref, dsk_ref, bre_ref, bim_ref, cre_ref, cim_ref,
               wg_ref, wu_ref, wd_ref, o_ref,
               par_ref, carry_ref, xnp_ref, u_ref, h_ref, act_ref, ys_ref):
        b = pl.program_id(0)

        @pl.when(b == 0)
        def _setup():
            lre = lre_ref[...].astype(f32).reshape(1, P)
            lim = lim_ref[...].astype(f32).reshape(1, P)
            dt = _rb(jnp.exp(ldt_ref[...].astype(f32).reshape(1, P)))
            a = dt * lre
            th = dt * lim
            mag = jnp.exp(a)
            lr = mag * jnp.cos(th)
            li = mag * jnp.sin(th)
            nr = lr - 1.0
            den = lre * lre + lim * lim
            cr = (nr * lre + li * lim) / den
            ci = (li * lre - nr * lim) / den
            def put(r, v):
                par_ref[r] = jnp.broadcast_to(v, (8, P))
            put(0, lr); put(1, li)
            put(2, 2.0 * cr); put(3, 2.0 * ci)
            pr, pi = lr, li
            n = 1
            while n < Tc:
                pr, pi = pr * pr - pi * pi, 2.0 * pr * pi
                n *= 2
            assert n == Tc
            put(4, pr); put(5, pi)
            pr, pi = pr * pr - pi * pi, 2.0 * pr * pi
            put(6, pr); put(7, pi)
            pr, pi = pr * pr - pi * pi, 2.0 * pr * pi
            put(8, pr); put(9, pi)
            put(10, dsk_ref[...].astype(f32).reshape(1, D))
            carry_ref[...] = jnp.zeros_like(carry_ref)

        dsk = par_ref[10][0:1, :]
        eps = np.float32(np.asarray(1e-5, dtype=jnp.bfloat16))
        def ln(rows):
            x = x_ref[rows, :].astype(f32)
            mean = jnp.sum(x, axis=-1, keepdims=True) * (1.0 / D)
            xc = x - mean
            var = jnp.sum(xc * xc, axis=-1, keepdims=True) * (1.0 / D)
            q = _rb(jnp.sqrt(_rb(_rb(var) + eps)))
            xn = _rb(x - _rb(mean)) * (1.0 / q)
            return x, xn
        for m in range(Tc // 16):
            for s in range(4):
                ra = pl.ds(2 * s * Tc + 16 * m, 16)
                rb_ = pl.ds((2 * s + 1) * Tc + 16 * m, 16)
                xa, na = ln(ra)
                xb, nb = ln(rb_)
                w = pltpu.pack_elementwise([na, nb], packed_dtype=bf16)
                for k in range(4):
                    xnp_ref[k, pl.ds(64 * m + s, 16, stride=4), :] = w[:, 128 * k:128 * (k + 1)]
                na_r = pltpu.unpack_elementwise(w, index=0, packed_dtype=bf16, unpacked_dtype=f32)
                nb_r = pltpu.unpack_elementwise(w, index=1, packed_dtype=bf16, unpacked_dtype=f32)
                o_ref[ra, :] = xa + na_r * dsk
                o_ref[rb_, :] = xb + nb_r * dsk

        xnb = xnp_ref.bitcast(bf16)
        xn = jnp.concatenate([xnb[k] for k in range(4)], axis=1)

        u_ref[:, 0:P] = jax.lax.dot_general(xn, bre_ref[...], NT, preferred_element_type=f32)
        u_ref[:, P:2 * P] = jax.lax.dot_general(xn, bim_ref[...], NT, preferred_element_type=f32)

        c1 = np.float32(np.sqrt(2.0 / np.pi))
        c2 = np.float32(np.sqrt(2.0 / np.pi) * 0.044715)
        cols = [(j * 256, 256) for j in range(F // 256)] + [((F // 256) * 256, F % 256)]
        for (c0, cw) in cols:
            g = jax.lax.dot_general(xn, wg_ref[c0:c0 + cw, :], NT, preferred_element_type=f32)
            up = jax.lax.dot_general(xn, wu_ref[c0:c0 + cw, :], NT, preferred_element_type=f32)
            t = jnp.tanh(g * (c1 + c2 * (g * g)))
            act_ref[:, c0:c0 + cw] = ((g * up) * (0.5 * t + 0.5)).astype(bf16)

        sub = jax.lax.broadcasted_iota(jnp.int32, (8, 128), 0)
        for k in range(4):
            ln_ = slice(128 * k, 128 * (k + 1))
            li_ = slice(P + 128 * k, P + 128 * (k + 1))
            lr = par_ref[0, :, ln_]; li = par_ref[1, :, ln_]
            gr = u_ref[0:8, ln_]; gi = u_ref[0:8, li_]
            for i in range(1, Tc):
                r = pl.ds(8 * i, 8)
                gr, gi = lr * gr - li * gi + u_ref[r, ln_], lr * gi + li * gr + u_ref[r, li_]
            cr_ = carry_ref[0, :, ln_]; ci_ = carry_ref[1, :, ln_]
            pr = par_ref[4, :, ln_]; pi = par_ref[5, :, ln_]
            ar, ai = _cmul(pr, pi, cr_, ci_)
            first = sub == 0
            sr = gr + jnp.where(first, ar, 0.0)
            si = gi + jnp.where(first, ai, 0.0)
            for (sh, row) in ((1, 4), (2, 6), (4, 8)):
                pr = par_ref[row, :, ln_]; pi = par_ref[row + 1, :, ln_]
                tr = pltpu.roll(sr, sh, 0); ti = pltpu.roll(si, sh, 0)
                ar, ai = _cmul(pr, pi, tr, ti)
                ok = sub >= sh
                sr = sr + jnp.where(ok, ar, 0.0)
                si = si + jnp.where(ok, ai, 0.0)
            hr = jnp.where(first, cr_, pltpu.roll(sr, 1, 0))
            hi = jnp.where(first, ci_, pltpu.roll(si, 1, 0))
            carry_ref[0, :, ln_] = jnp.broadcast_to(sr[7:8, :], (8, 128))
            carry_ref[1, :, ln_] = jnp.broadcast_to(si[7:8, :], (8, 128))
            kr = par_ref[2, :, ln_]; ki = par_ref[3, :, ln_]
            for i in range(0, Tc, 2):
                outs_r = []; outs_i = []
                for ii in (i, i + 1):
                    r = pl.ds(8 * ii, 8)
                    hr, hi = lr * hr - li * hi + u_ref[r, ln_], lr * hi + li * hr + u_ref[r, li_]
                    outs_r.append(kr * hr - ki * hi)
                    outs_i.append(-(kr * hi + ki * hr))
                h_ref[pl.ds(8 * i, 16), ln_] = jnp.concatenate(outs_r, axis=0).astype(bf16)
                h_ref[pl.ds(8 * i, 16), li_] = jnp.concatenate(outs_i, axis=0).astype(bf16)

        acc = jnp.dot(act_ref[...], wd_ref[...], preferred_element_type=f32)
        acc += jax.lax.dot_general(h_ref[:, 0:P], cre_ref[...], NT, preferred_element_type=f32)
        acc += jax.lax.dot_general(h_ref[:, P:2 * P], cim_ref[...], NT, preferred_element_type=f32)
        for k in range(4):
            for i in range(Tc):
                ys_ref[k, pl.ds(i, 8, stride=SY), :] = acc[8 * i:8 * i + 8, 128 * k:128 * (k + 1)]
        for k in range(4):
            for j in range(8):
                o_ref[pl.ds(j * Tc, Tc), 128 * k:128 * (k + 1)] += ys_ref[k, pl.ds(j * SY, Tc), :]

    def full(shape):
        return pl.BlockSpec(shape, lambda b: (0,) * len(shape))

    def run(x, lre, lim, ldt, dsk, bre, bim, cre, cim, wg, wu, wd):
        return pl.pallas_call(
            kernel,
            grid=(NB,),
            in_specs=[pl.BlockSpec((Tb, D), lambda b: (b, 0)),
                      full((P,)), full((P,)), full((P,)), full((D,)),
                      full((P, D)), full((P, D)), full((D, P)), full((D, P)),
                      full((F, D)), full((F, D)), full((F, D))],
            out_specs=pl.BlockSpec((Tb, D), lambda b: (b, 0)),
            out_shape=jax.ShapeDtypeStruct((L, D), f32),
            scratch_shapes=[
                pltpu.VMEM((11, 8, P), f32),
                pltpu.VMEM((2, 8, P), f32),
                pltpu.VMEM((4, Tb // 2, 128), jnp.int32),
                pltpu.VMEM((Tb, 2 * P), f32),
                pltpu.VMEM((Tb, 2 * P), bf16),
                pltpu.VMEM((Tb, F), bf16),
                pltpu.VMEM((4, 8 * SY, 128), f32),
            ],
            compiler_params=pltpu.CompilerParams(dimension_semantics=("arbitrary",), vmem_limit_bytes=100 * 2**20),
            interpret=interpret,
        )(x, lre, lim, ldt, dsk, bre, bim, cre, cim, wg, wu, wd)
    return run

_run = make(512)


@jax.jit
def pallas_parallel_sum__ssm_conv_s5__geglu_ffn__prompt_kernel(
    A_x, A_Lambda_re, A_Lambda_im, A_B_re, A_B_im, A_C_re, A_C_im, A_log_dt, A_Dskip,
    B_x, B_w_gate, B_w_up, B_w_down,
):
    out = _run(A_x.reshape(L, D), A_Lambda_re, A_Lambda_im, A_log_dt, A_Dskip, A_B_re, A_B_im, A_C_re, A_C_im,
               B_w_gate.T, B_w_up.T, B_w_down)
    return out.reshape(1, L, D)
```

```python
import jax
import jax.numpy as jnp
import numpy as np
from jax.experimental import pallas as pl
from jax.experimental.pallas import tpu as pltpu


L, D, P, F = 2048, 512, 512, 1376
f32, bf16 = jnp.float32, jnp.bfloat16
NT = (((1,), (1,)), ((), ()))

def _rb(v):
    return v.astype(bf16).astype(f32)

def _cmul(ar, ai, br, bi):
    return ar * br - ai * bi, ar * bi + ai * br

def make(Tb=512, head="sep", CG=256, gsplit=2, sj=0, dw=128, lnpos="before", dm=512, um=512, inter=True, scopes=False, lg=1, bsplit=True, osplit=1, opq=""):
    NB = L // Tb
    Tc = Tb // 8
    SY = Tc + 1
    cols = [(j * CG, CG) for j in range(F // CG)] + ([((F // CG) * CG, F % CG)] if F % CG else [])
    NG = len(cols)

    def kernel(x_hbm, lre_hbm, lim_hbm, ldt_hbm, dsk_hbm, bre_hbm, bim_hbm, cre_hbm, cim_hbm,
               wg_hbm, wu_hbm, wd_hbm, o_hbm,
               x_v, p1_v, bre_v, bim_v, cre_v, cim_v, wg_v, wu_v, wd_v, o_v,
               par_st, xnp_ref, u_ref, h_ref, act_ref, ys_ref,
               sem_in, sem_o, sem_z):
        import contextlib
        def sc(name):
            return jax.named_scope(name) if scopes else contextlib.nullcontext()
        _n = [0]
        def mk(src, dst):
            _n[0] += 1
            return pltpu.make_async_copy(src, dst, sem_in.at[_n[0] - 1])
        cp_p = [mk(s_, p1_v[i]) for i, s_ in enumerate((lre_hbm, lim_hbm, ldt_hbm, dsk_hbm))]
        cp_x = [None] * NB
        def mkx(b):
            cp_x[b] = mk(x_hbm.at[pl.ds(b * Tb, Tb), :], x_v.at[pl.ds(b * Tb, Tb), :])
            return cp_x[b]
        for c in cp_p: c.start()
        mkx(0).start()
        cp_b = [mk(bre_hbm, bre_v), mk(bim_hbm, bim_v)]
        for c in cp_b: c.start()
        cp_g = []
        for j, (c0, cw) in enumerate(cols):
            cp_g.append((mk(wg_hbm.at[pl.ds(c0, cw), :], wg_v.at[pl.ds(c0, cw), :]),
                         mk(wu_hbm.at[pl.ds(c0, cw), :], wu_v.at[pl.ds(c0, cw), :])))
            cp_g[j][0].start(); cp_g[j][1].start()
            if j == gsplit - 1 and NB > 1:
                mkx(1).start()
        cp_d = mk(wd_hbm, wd_v)
        cp_d.start()
        cp_c = [mk(cre_hbm, cre_v), mk(cim_hbm, cim_v)]
        for c in cp_c: c.start()
        for b in range(2, NB):
            mkx(b).start()

        z = pl.semaphore_read(sem_z)
        with sc('w_p'):
            for c in cp_p: c.wait()
        lre = p1_v[0][...].astype(f32).reshape(1, P)
        lim = p1_v[1][...].astype(f32).reshape(1, P)
        dt = _rb(jnp.exp(p1_v[2][...].astype(f32).reshape(1, P)))
        a = dt * lre
        th = dt * lim
        mag = jnp.exp(a)
        lr = mag * jnp.cos(th)
        li = mag * jnp.sin(th)
        nr = lr - 1.0
        den = lre * lre + lim * lim
        cr = (nr * lre + li * lim) / den
        ci = (li * lre - nr * lim) / den
        def put(r, v):
            par_st[r] = jnp.broadcast_to(v, (8, P))
        put(0, lr); put(1, li)
        put(2, 2.0 * cr); put(3, 2.0 * ci); put(11, -2.0 * cr); put(12, -2.0 * ci)
        pr, pi = lr, li
        n = 1
        while n < Tc:
            pr, pi = pr * pr - pi * pi, 2.0 * pr * pi
            n *= 2
        assert n == Tc
        put(4, pr); put(5, pi)
        pr, pi = pr * pr - pi * pi, 2.0 * pr * pi
        put(6, pr); put(7, pi)
        pr, pi = pr * pr - pi * pi, 2.0 * pr * pi
        put(8, pr); put(9, pi)
        put(10, p1_v[3][...].astype(f32).reshape(1, D))

        def parld(r):
            return par_st[r + z] if 'p' in opq else par_st[r]
        eps = np.float32(np.asarray(1e-5, dtype=jnp.bfloat16))
        c1 = np.float32(np.sqrt(2.0 / np.pi))
        c2 = np.float32(np.sqrt(2.0 / np.pi) * 0.044715)
        sub = jax.lax.broadcasted_iota(jnp.int32, (8, 128), 0)

        def ln_stage(b, ms=None):
            xnw = xnp_ref.bitcast(jnp.int32)
            dsk = parld(10)[0:1, :]
            link = [None, 0]
            def ln(rows, inv):
                x = x_v[rows, :].astype(f32)
                mean = jnp.sum(x, axis=-1, keepdims=True) * inv
                xc = x - mean
                var = jnp.sum(xc * xc, axis=-1, keepdims=True) * (1.0 / D)
                q = _rb(jnp.sqrt(_rb(_rb(var) + eps)))
                xn = _rb(x - _rb(mean)) * (1.0 / q)
                return x, xn
            for m in (range(Tc // 16) if ms is None else ms):
                for s in range(4):
                    ra = pl.ds(b * Tb + 2 * s * Tc + 16 * m, 16)
                    rb_ = pl.ds(b * Tb + (2 * s + 1) * Tc + 16 * m, 16)
                    inv = 1.0 / D
                    if link[0] is not None:
                        one = jnp.where((link[0] | 1) == 0, 0.0, 1.0 / D).astype(f32)[:, 0:1]
                        inv = jnp.concatenate([one, one], axis=0)
                    xa, na = ln(ra, inv)
                    xb, nb = ln(rb_, inv)
                    w = pltpu.pack_elementwise([na, nb], packed_dtype=bf16)
                    link[1] += 1
                    if lg and b > 0 and link[1] % lg == 0:
                        link[0] = w[0:8, 0:128]
                    for k in range(4):
                        xnw[b, k, pl.ds(64 * m + s, 16, stride=4), :] = w[:, 128 * k:128 * (k + 1)]
                    na_r = pltpu.unpack_elementwise(w, index=0, packed_dtype=bf16, unpacked_dtype=f32)
                    nb_r = pltpu.unpack_elementwise(w, index=1, packed_dtype=bf16, unpacked_dtype=f32)
                    o_v[ra, :] = xa + na_r * dsk
                    o_v[rb_, :] = xb + nb_r * dsk

        def get_xn(b):
            return jnp.concatenate([xnp_ref[b, k] for k in range(4)], axis=1)

        def bu_stage(b, m0=0, mw=None, parts=(0, 1)):
            mw = Tb if mw is None else mw
            rs = pl.ds(m0, mw)
            xn = jnp.concatenate([xnp_ref[b, k, rs, :] for k in range(4)], axis=1)
            if 0 in parts:
                u_ref[b, rs, 0:P] = jax.lax.dot_general(xn, bre_v[...], NT, preferred_element_type=f32)
            if 1 in parts:
                u_ref[b, rs, P:2 * P] = jax.lax.dot_general(xn, bim_v[...], NT, preferred_element_type=f32)

        def ffn_up(b, j):
            c0, cw = cols[j]
            for m0 in range(0, Tb, um):
                rs = pl.ds(m0, um)
                xn = jnp.concatenate([xnp_ref[b, k, rs, :] for k in range(4)], axis=1)
                g = jax.lax.dot_general(xn, wg_v[c0:c0 + cw, :], NT, preferred_element_type=f32)
                up = jax.lax.dot_general(xn, wu_v[c0:c0 + cw, :], NT, preferred_element_type=f32)
                t = jnp.tanh(g * (c1 + c2 * (g * g)))
                act_ref[b, rs, c0:c0 + cw] = ((g * up) * (0.5 * t + 0.5)).astype(bf16)

        carry = [None] * 4

        def scan_stage(b, k):
            ln_ = slice(128 * k, 128 * (k + 1))
            li_ = slice(P + 128 * k, P + 128 * (k + 1))
            lr = parld(0)[:, ln_]; li = parld(1)[:, ln_]
            bu = b + z if 'u' in opq else b
            gr = u_ref[bu, 0:8, ln_]; gi = u_ref[bu, 0:8, li_]
            for i in range(1, Tc):
                r = pl.ds(8 * i, 8)
                gr, gi = lr * gr - li * gi + u_ref[bu, r, ln_], lr * gi + li * gr + u_ref[bu, r, li_]
            first = sub == 0
            sr, si = gr, gi
            if carry[k] is not None:
                cr_, ci_ = carry[k]
                ar, ai = _cmul(parld(4)[:, ln_], parld(5)[:, ln_], cr_, ci_)
                sr = sr + jnp.where(first, ar, 0.0)
                si = si + jnp.where(first, ai, 0.0)
            for (sh, row) in ((1, 4), (2, 6), (4, 8)):
                pr = parld(row)[:, ln_]; pi = parld(row + 1)[:, ln_]
                tr = pltpu.roll(sr, sh, 0); ti = pltpu.roll(si, sh, 0)
                ar, ai = _cmul(pr, pi, tr, ti)
                ok = sub >= sh
                sr = sr + jnp.where(ok, ar, 0.0)
                si = si + jnp.where(ok, ai, 0.0)
            if carry[k] is not None:
                hr = jnp.where(first, cr_, pltpu.roll(sr, 1, 0))
                hi = jnp.where(first, ci_, pltpu.roll(si, 1, 0))
            else:
                hr = jnp.where(first, 0.0, pltpu.roll(sr, 1, 0))
                hi = jnp.where(first, 0.0, pltpu.roll(si, 1, 0))
            carry[k] = (jnp.broadcast_to(sr[7:8, :], (8, 128)), jnp.broadcast_to(si[7:8, :], (8, 128)))
            kr = parld(2)[:, ln_]; ki = parld(3)[:, ln_]; nkr = parld(11)[:, ln_]; nki = parld(12)[:, ln_]
            for i in range(0, Tc, 2):
                outs_r = []; outs_i = []
                for ii in (i, i + 1):
                    r = pl.ds(8 * ii, 8)
                    hr, hi = lr * hr - li * hi + u_ref[bu, r, ln_], lr * hi + li * hr + u_ref[bu, r, li_]
                    outs_r.append(kr * hr - ki * hi)
                    outs_i.append(nkr * hi + nki * hr)
                h_ref[b, pl.ds(8 * i, 16), ln_] = jnp.concatenate(outs_r, axis=0).astype(bf16)
                h_ref[b, pl.ds(8 * i, 16), li_] = jnp.concatenate(outs_i, axis=0).astype(bf16)

        def down_stage(b, ks=range(4), dw=128):
            for k in ks:
                cs = slice(dw * k, dw * (k + 1))
                for m0 in range(0, Tb, dm):
                    rs = pl.ds(m0, dm)
                    ba = b + z if 'a' in opq else b
                    bh = b + z if 'h' in opq else b
                    acc = jnp.dot(act_ref[ba, rs, :], wd_v[:, cs], preferred_element_type=f32)
                    acc += jax.lax.dot_general(h_ref[bh, rs, 0:P], cre_v[cs, :], NT, preferred_element_type=f32)
                    acc += jax.lax.dot_general(h_ref[bh, rs, P:2 * P], cim_v[cs, :], NT, preferred_element_type=f32)
                    for kk in range(dw // 128):
                        for i in range(dm // 8):
                            ys_ref[b, k * (dw // 128) + kk, pl.ds(m0 // 8 + i, 8, stride=SY), :] = acc[8 * i:8 * i + 8, 128 * kk:128 * (kk + 1)]

        cp_o = []
        def fin_stage(b, ks=range(4), ow=1):
            for j in range(8):
                rows = pl.ds(pl.multiple_of(b * Tb + j * Tc + (8 * z if 'o' in opq else 0), 8), Tc)
                for k in ks:
                    o_v[rows, 128 * k:128 * (k + 1)] += ys_ref[b, k, pl.ds(j * SY, Tc), :]
            rows = pl.ds(b * Tb, Tb)
            cs = pl.ds(128 * ks[0], 128 * len(ks))
            c = pltpu.make_async_copy(o_v.at[rows, cs], o_hbm.at[rows, cs], sem_o.at[len(cp_o)])
            c.start()
            cp_o.append(c)

        def wait_g(js):
            for j in js:
                cp_g[j][0].wait(); cp_g[j][1].wait()
        GS = gsplit
        with sc("w_x0"):
            cp_x[0].wait()
        with sc("ln0"):
            ln_stage(0)
        if bsplit:
            with sc("w_Bre"):
                cp_b[0].wait()
            with sc("bu0re"):
                bu_stage(0, parts=(0,))
            with sc("w_Bim"):
                cp_b[1].wait()
            with sc("bu0im"):
                bu_stage(0, parts=(1,))
        else:
            with sc("w_B"):
                cp_b[0].wait(); cp_b[1].wait()
            with sc("bu0"):
                bu_stage(0)
        for b in range(NB):
            if b > 0 and not inter:
                bu_stage(b)
            if b > 0 and not osplit: fin_stage(b - 1)
            if b == 0:
                with sc('w_g1'):
                    wait_g(range(GS))
            for j in range(NG):
                if b == 0 and j == GS:
                    with sc('w_g2'):
                        wait_g(range(GS, NG))
                        if NB > 1: cp_x[1].wait()
                ffn_up(b, j)
                if j >= sj and j < sj + 4: scan_stage(b, j - sj)
            if b == 0:
                with sc('w_d'):
                    cp_d.wait(); cp_c[0].wait(); cp_c[1].wait()
                    for bb in range(2, NB): cp_x[bb].wait()
            nd = 512 // dw
            NM = Tc // 16
            for k in range(nd):
                ms = range(k * NM // nd, (k + 1) * NM // nd)
                if b + 1 < NB: ln_stage(b + 1, ms)
                down_stage(b, [k], dw)
                if inter and b + 1 < NB and len(ms): bu_stage(b + 1, ms[0] * 128, len(ms) * 128)
                if osplit:
                    kk = list(range(k * dw // 128, (k + 1) * dw // 128))
                    if b == NB - 1 or osplit == 2:
                        fin_stage(b, kk)
                    elif k == nd - 1:
                        fin_stage(b)
        if not osplit:
            with sc('fin_last'):
                fin_stage(NB - 1)
        with sc('w_out'):
            for c in cp_o: c.wait()

    def run(x, lre, lim, ldt, dsk, bre, bim, cre, cim, wg, wu, wd):
        anyspec = pl.BlockSpec(memory_space=pl.ANY)
        return pl.pallas_call(
            kernel,
            in_specs=[anyspec] * 12,
            out_specs=anyspec,
            out_shape=jax.ShapeDtypeStruct((L, D), f32),
            scratch_shapes=[
                pltpu.VMEM((L, D), bf16),
                [pltpu.VMEM((P,), bf16)] * 4,
                pltpu.VMEM((P, D), bf16), pltpu.VMEM((P, D), bf16),
                pltpu.VMEM((D, P), bf16), pltpu.VMEM((D, P), bf16),
                pltpu.VMEM((F, D), bf16), pltpu.VMEM((F, D), bf16), pltpu.VMEM((F, D), bf16),
                pltpu.VMEM((L, D), f32),
                pltpu.VMEM((13, 8, P), f32),
                pltpu.VMEM((NB, 4, Tb, 128), bf16),
                pltpu.VMEM((NB, Tb, 2 * P), f32),
                pltpu.VMEM((NB, Tb, 2 * P), bf16),
                pltpu.VMEM((NB, Tb, F), bf16),
                pltpu.VMEM((NB, 4, 8 * SY, 128), f32),
                pltpu.SemaphoreType.DMA((4 + NB + 5 + 2 * NG,)), pltpu.SemaphoreType.DMA((4 * NB,)), pltpu.SemaphoreType.REGULAR,
            ],
            compiler_params=pltpu.CompilerParams(vmem_limit_bytes=100 * 2**20),
        )(x, lre, lim, ldt, dsk, bre, bim, cre, cim, wg, wu, wd)
    return run

_run = make(512, dw=128, dm=512, lg=1, opq='u')


@jax.jit
def pallas_parallel_sum__ssm_conv_s5__geglu_ffn__prompt_kernel(
    A_x, A_Lambda_re, A_Lambda_im, A_B_re, A_B_im, A_C_re, A_C_im, A_log_dt, A_Dskip,
    B_x, B_w_gate, B_w_up, B_w_down,
):
    out = _run(A_x.reshape(L, D), A_Lambda_re, A_Lambda_im, A_log_dt, A_Dskip, A_B_re, A_B_im, A_C_re, A_C_im,
               B_w_gate.T, B_w_up.T, B_w_down)
    return out.reshape(1, L, D)
```

```python
import jax
import jax.numpy as jnp
import numpy as np
from jax.experimental import pallas as pl
from jax.experimental.pallas import tpu as pltpu

L, D, P, F = 2048, 512, 512, 1376
f32, bf16 = jnp.float32, jnp.bfloat16
NT = (((1,), (1,)), ((), ()))

TB = 512
NB = L // TB
TC = TB // 8
SY = TC + 1
COLS = [(c, min(256, F - c)) for c in range(0, F, 256)]
GSPLIT = 2
BGROUPS = (((0, 0, 128),), ((0, 128, 256),), ((0, 384, 128), (1, 0, 512)))
G_X0, G_X1, G_B0, G_G1, G_G2, G_D, G_OUT = 0, 1, 2, 5, 6, 7, 8


def _cmul(ar, ai, br, bi):
    return ar * br - ai * bi, ar * bi + ai * br


def _kernel(x_hbm, lre_hbm, lim_hbm, ldt_hbm, dsk_hbm, bre_hbm, bim_hbm, cre_hbm, cim_hbm,
            wg_hbm, wu_hbm, wd_hbm, o_hbm,
            x_v, p1_v, bre_v, bim_v, cre_v, cim_v, wg_v, wu_v, wd_v, o_v,
            par_ref, xnp_ref, u_ref, h_ref, act_ref, ys_ref, sem, sem_z):
    groups = {}

    def dma(g, src, dst, rows=None):
        if rows is not None:
            src, dst = src.at[pl.ds(*rows), :], dst.at[pl.ds(*rows), :]
        c = pltpu.make_async_copy(src, dst, sem.at[g])
        c.start()
        groups.setdefault(g, []).append(c)

    def wait(g):
        for c in groups.pop(g):
            c.wait()

    b_hbm, b_v = (bre_hbm, bim_hbm), (bre_v, bim_v)
    dma(G_X0, x_hbm, x_v, (0, TB // 2))
    dma(G_X1, x_hbm, x_v, (TB // 2, TB // 2))
    for gi, parts in enumerate(BGROUPS):
        for part, r0, nr in parts:
            dma(G_B0 + gi, b_hbm[part], b_v[part], None if nr == P else (r0, nr))
        if gi == 1:
            for i, src in enumerate((lre_hbm, lim_hbm, ldt_hbm, dsk_hbm)):
                dma(G_B0 + gi, src, p1_v[i])
    r1 = COLS[GSPLIT][0]
    dma(G_G1, wg_hbm, wg_v, (0, r1))
    dma(G_G1, wu_hbm, wu_v, (0, r1))
    dma(G_G2, wg_hbm, wg_v, (r1, F - r1))
    dma(G_G2, wu_hbm, wu_v, (r1, F - r1))
    dma(G_D, wd_hbm, wd_v)
    dma(G_D, cre_hbm, cre_v)
    dma(G_D, cim_hbm, cim_v)
    dma(G_D, x_hbm, x_v, (TB, L - TB))

    z = pl.semaphore_read(sem_z)

    eps = np.float32(1e-5)
    c1 = np.float32(np.sqrt(2.0 / np.pi))
    c2 = np.float32(np.sqrt(2.0 / np.pi) * 0.044715)
    sub = jax.lax.broadcasted_iota(jnp.int32, (8, 128), 0)

    def ln_stage(b, pieces, linked):
        xnw = xnp_ref.bitcast(jnp.int32)
        link = None

        def ln(rows, inv):
            x = x_v[rows, :].astype(f32)
            xc = x - jnp.sum(x, axis=-1, keepdims=True) * inv
            var = jnp.sum(xc * xc, axis=-1, keepdims=True) * (1.0 / D)
            return xc * jax.lax.rsqrt(var + eps)

        for m, s in pieces:
            inv = 1.0 / D
            if link is not None:
                one = jnp.where((link | 1) == 0, 0.0, 1.0 / D).astype(f32)[:, 0:1]
                inv = jnp.concatenate([one, one], axis=0)
            na = ln(pl.ds(b * TB + 2 * s * TC + 16 * m, 16), inv)
            nb = ln(pl.ds(b * TB + (2 * s + 1) * TC + 16 * m, 16), inv)
            w = pltpu.pack_elementwise([na, nb], packed_dtype=bf16)
            if linked:
                link = w[0:8, 0:128]
            for k in range(4):
                xnw[b, k, pl.ds(64 * m + s, 16, stride=4), :] = w[:, 128 * k:128 * (k + 1)]

    def setup():
        lre = p1_v[0][...].astype(f32).reshape(1, P)
        lim = p1_v[1][...].astype(f32).reshape(1, P)
        dt = jnp.exp(p1_v[2][...].astype(f32).reshape(1, P)).astype(bf16).astype(f32)
        a = dt * lre
        th = dt * lim
        mag = jnp.exp(a)
        lr = mag * jnp.cos(th)
        li = mag * jnp.sin(th)
        nr = lr - 1.0
        den = lre * lre + lim * lim
        cr = (nr * lre + li * lim) / den
        ci = (li * lre - nr * lim) / den

        def put(r, v):
            par_ref[r] = jnp.broadcast_to(v, (8, P))
        put(0, lr); put(1, li)
        put(2, 2.0 * cr); put(3, 2.0 * ci); put(11, -2.0 * cr); put(12, -2.0 * ci)
        pr, pi = lr, li
        for _ in range(TC.bit_length() - 1):
            pr, pi = pr * pr - pi * pi, 2.0 * pr * pi
        put(4, pr); put(5, pi)
        pr, pi = pr * pr - pi * pi, 2.0 * pr * pi
        put(6, pr); put(7, pi)
        pr, pi = pr * pr - pi * pi, 2.0 * pr * pi
        put(8, pr); put(9, pi)
        put(10, p1_v[3][...].astype(f32).reshape(1, D))

    def xn_of(b):
        return jnp.concatenate([xnp_ref[b, k] for k in range(4)], axis=1)

    def bu_stage(b, parts=((0, 0, P), (1, 0, P))):
        xn = xn_of(b)
        for part, r0, nr in parts:
            v = jax.lax.dot_general(xn, b_v[part][r0:r0 + nr, :], NT, preferred_element_type=f32)
            for t in range(nr // 128):
                c = 128 * (2 * (r0 // 128 + t) + part)
                u_ref[b, :, c:c + 128] = v[:, 128 * t:128 * (t + 1)]

    def ffn_up(b, j):
        c0, cw = COLS[j]
        xn = xn_of(b)
        g = jax.lax.dot_general(xn, wg_v[c0:c0 + cw, :], NT, preferred_element_type=f32)
        up = jax.lax.dot_general(xn, wu_v[c0:c0 + cw, :], NT, preferred_element_type=f32)
        t = jnp.tanh(g * (c1 + c2 * (g * g)))
        act_ref[b, :, c0:c0 + cw] = ((g * up) * (0.5 * t + 0.5)).astype(bf16)

    carry = [None] * 4

    def scan_stage(b, k):
        cs = slice(128 * k, 128 * (k + 1))
        ur = slice(256 * k, 256 * k + 128)
        ui = slice(256 * k + 128, 256 * k + 256)
        bz = b + z
        lr = par_ref[0][:, cs]; li = par_ref[1][:, cs]
        sr = u_ref[bz, 0:8, ur]; si = u_ref[bz, 0:8, ui]
        for i in range(1, TC):
            r = pl.ds(8 * i, 8)
            sr, si = lr * sr - li * si + u_ref[bz, r, ur], lr * si + li * sr + u_ref[bz, r, ui]
        first = sub == 0
        if carry[k] is not None:
            c_r, c_i = carry[k]
            ar, ai = _cmul(par_ref[4][:, cs], par_ref[5][:, cs], c_r, c_i)
            sr = sr + jnp.where(first, ar, 0.0)
            si = si + jnp.where(first, ai, 0.0)
        else:
            c_r = c_i = 0.0
        for sh, row in ((1, 4), (2, 6), (4, 8)):
            tr = pltpu.roll(sr, sh, 0); ti = pltpu.roll(si, sh, 0)
            ar, ai = _cmul(par_ref[row][:, cs], par_ref[row + 1][:, cs], tr, ti)
            ok = sub >= sh
            sr = sr + jnp.where(ok, ar, 0.0)
            si = si + jnp.where(ok, ai, 0.0)
        hr = jnp.where(first, c_r, pltpu.roll(sr, 1, 0))
        hi = jnp.where(first, c_i, pltpu.roll(si, 1, 0))
        carry[k] = (jnp.broadcast_to(sr[7:8, :], (8, 128)), jnp.broadcast_to(si[7:8, :], (8, 128)))
        kr = par_ref[2][:, cs]; ki = par_ref[3][:, cs]
        nkr = par_ref[11][:, cs]; nki = par_ref[12][:, cs]
        for i in range(0, TC, 2):
            outs_r, outs_i = [], []
            for ii in (i, i + 1):
                r = pl.ds(8 * ii, 8)
                hr, hi = lr * hr - li * hi + u_ref[b, r, ur], lr * hi + li * hr + u_ref[b, r, ui]
                outs_r.append(kr * hr - ki * hi)
                outs_i.append(nkr * hi + nki * hr)
            h_ref[b, pl.ds(8 * i, 16), cs] = jnp.concatenate(outs_r, axis=0).astype(bf16)
            h_ref[b, pl.ds(8 * i, 16), P + 128 * k:P + 128 * (k + 1)] = (
                jnp.concatenate(outs_i, axis=0).astype(bf16))

    def down_stage(b, k):
        cs = slice(128 * k, 128 * (k + 1))
        acc = jnp.dot(act_ref[b], wd_v[:, cs], preferred_element_type=f32)
        acc += jax.lax.dot_general(h_ref[b, :, 0:P], cre_v[cs, :], NT, preferred_element_type=f32)
        acc += jax.lax.dot_general(h_ref[b, :, P:2 * P], cim_v[cs, :], NT, preferred_element_type=f32)
        acc += xnp_ref[b, k].astype(f32) * par_ref[10][0:1, cs]
        for i in range(TC):
            ys_ref[b, k, pl.ds(i, 8, stride=SY), :] = acc[8 * i:8 * i + 8, :]

    out_cp = []

    def fin_stage(b, ks):
        for j in range(8):
            rows = pl.ds(b * TB + j * TC, TC)
            for k in ks:
                cs = slice(128 * k, 128 * (k + 1))
                o_v[rows, cs] = x_v[rows, cs].astype(f32) + ys_ref[b, k, pl.ds(j * SY, TC), :]
        rows = pl.ds(b * TB, TB)
        cs = pl.ds(128 * ks[0], 128 * len(ks))
        c = pltpu.make_async_copy(o_v.at[rows, cs], o_hbm.at[rows, cs], sem.at[G_OUT])
        c.start()
        out_cp.append(c)

    for i in range(2):
        wait(G_X0 + i)
        ln_stage(0, [(m, s) for s in (2 * i, 2 * i + 1) for m in range(TC // 16)], False)
    for gi, parts in enumerate(BGROUPS):
        wait(G_B0 + gi)
        if gi == 1:
            setup()
        bu_stage(0, parts)
    for b in range(NB):
        if b > 0:
            bu_stage(b)
        else:
            wait(G_G1)
        for j in range(len(COLS)):
            if b == 0 and j == GSPLIT:
                wait(G_G2)
            ffn_up(b, j)
            if j < 4:
                scan_stage(b, j)
        if b == 0:
            wait(G_D)
        for k in range(4):
            if b + 1 < NB:
                ln_stage(b + 1, [(k, s) for s in range(4)], True)
            down_stage(b, k)
            if b == NB - 1:
                fin_stage(b, [k])
            elif k == 3:
                fin_stage(b, [0, 1, 2, 3])
    for c in out_cp:
        c.wait()


@jax.jit
def pallas_parallel_sum__ssm_conv_s5__geglu_ffn__prompt_kernel(
    A_x: jax.Array,
    A_Lambda_re: jax.Array,
    A_Lambda_im: jax.Array,
    A_B_re: jax.Array,
    A_B_im: jax.Array,
    A_C_re: jax.Array,
    A_C_im: jax.Array,
    A_log_dt: jax.Array,
    A_Dskip: jax.Array,
    B_x: jax.Array,
    B_w_gate: jax.Array,
    B_w_up: jax.Array,
    B_w_down: jax.Array,
):
    del B_x
    anyspec = pl.BlockSpec(memory_space=pl.ANY)
    out = pl.pallas_call(
        _kernel,
        in_specs=[anyspec] * 12,
        out_specs=anyspec,
        out_shape=jax.ShapeDtypeStruct((L, D), f32),
        scratch_shapes=[
            pltpu.VMEM((L, D), bf16),
            [pltpu.VMEM((P,), bf16)] * 4,
            pltpu.VMEM((P, D), bf16), pltpu.VMEM((P, D), bf16),
            pltpu.VMEM((D, P), bf16), pltpu.VMEM((D, P), bf16),
            pltpu.VMEM((F, D), bf16), pltpu.VMEM((F, D), bf16), pltpu.VMEM((F, D), bf16),
            pltpu.VMEM((L, D), f32),
            pltpu.VMEM((13, 8, P), f32),
            pltpu.VMEM((NB, 4, TB, 128), bf16),
            pltpu.VMEM((NB, TB, 2 * P), f32),
            pltpu.VMEM((NB, TB, 2 * P), bf16),
            pltpu.VMEM((NB, TB, F), bf16),
            pltpu.VMEM((NB, 4, 8 * SY, 128), f32),
            pltpu.SemaphoreType.DMA((G_OUT + 1,)),
            pltpu.SemaphoreType.REGULAR,
        ],
        compiler_params=pltpu.CompilerParams(vmem_limit_bytes=100 * 2**20),
    )(A_x.reshape(L, D), A_Lambda_re, A_Lambda_im, A_log_dt, A_Dskip, A_B_re, A_B_im, A_C_re, A_C_im,
      B_w_gate.T, B_w_up.T, B_w_down)
    return out.reshape(1, L, D)
```
